```python
import os as _os
_os.environ.setdefault("JAX_PLATFORMS", "cpu")
import jax
import jax.numpy as jnp

def _softmax(x, axis=-1):
    return jax.nn.softmax(x, axis=axis)
def _gelu(x):
    return jax.nn.gelu(x, approximate=True)
def _silu(x):
    return jax.nn.silu(x)
def _sigmoid(x):
    return jax.nn.sigmoid(x)
def _layernorm(x, axis=-1, eps=1e-5):
    m = jnp.mean(x, axis=axis, keepdims=True)
    v = jnp.var(x, axis=axis, keepdims=True)
    return (x - m) / jnp.sqrt(v + eps)
def _scatter_add(tgt, idx, src, axis=0):
    return tgt.at[idx].add(src)
def _segment_sum(src, seg, n):
    return jax.ops.segment_sum(src, seg, n)
class _Rng:
    def __init__(self, key):
        self._k = key
    def _next(self):
        self._k, sub = jax.random.split(self._k)
        return sub
    def normal(self, shape):
        return jax.random.normal(self._next(), shape, dtype=jnp.bfloat16)
    def randint(self, lo, hi, shape):
        return jax.random.randint(self._next(), shape, lo, hi, dtype=jnp.int32)
    def uniform(self, shape, lo=0.0, hi=1.0):
        return jax.random.uniform(self._next(), shape, jnp.bfloat16, lo, hi)
    def permutation(self, n):
        return jax.random.permutation(self._next(), n)


kernel_name = 'standalone__gqa_block_cached__near_ridge'

def setup_inputs():
    _rng = _Rng(jax.random.key(int.from_bytes(__import__("os").urandom(4), "little")))
    _w = (lambda a: (lambda t: t.astype(jnp.bfloat16) if jnp.issubdtype(t.dtype, jnp.floating) else t)(jnp.asarray(a)))
    B, Sq, D = 8, 80, 512
    Hq, Hkv, Sk, Dh = 32, 8, 2048, 128
    assert Hq % Hkv == 0, (Hq, Hkv)
    return {
        "x": _w((lambda *s: _rng.normal(s) * 0.8)(B, Sq, D)),
        "k_cache": _w((lambda *s: _rng.normal(s) * 0.8)(B, Hkv, Sk, Dh)),
        "v_cache": _w((lambda *s: _rng.normal(s) * 0.05)(B, Hkv, Sk, Dh)),
        "wq": _w((lambda *s: _rng.normal(s) * 0.8)(D, Hq * Dh) * (D ** -0.5)),
        "wo": _w((lambda *s: _rng.normal(s) * 0.05)(Hq * Dh, D) * ((Hq * Dh) ** -0.5)),
    }

def reference(x, k_cache, v_cache, wq, wo):
    B, Sq, D = x.shape
    Hq, Dh = 32, 128
    Hkv = k_cache.shape[1]
    rep = Hq // Hkv
    q = (lambda x, *d: x.transpose(*d))((x @ wq).reshape(B, Sq, Hq, Dh), 0, 2, 1, 3)
    k = jnp.repeat(k_cache, rep, axis=1)
    v = jnp.repeat(v_cache, rep, axis=1)
    scores = jnp.einsum("bhqd,bhkd->bhqk", q, k) * (Dh ** -0.5)
    p = _softmax(scores, axis=-1)
    o = jnp.einsum("bhqk,bhkd->bhqd", p, v)
    return (lambda x, *d: x.transpose(*d))(o, 0, 2, 1, 3).reshape(B, Sq, Hq * Dh) @ wo
```

```python
import functools
import math
import os
import jax
import jax.numpy as jnp
import jax.experimental.pallas as pl
import jax.experimental.pallas.tpu as pltpu

HQ = 32
RG = 16
NSPLIT = int(os.environ.get("NSPLIT", "2"))
PACE = int(os.environ.get("PACE", "72"))
NU = int(os.environ.get("NU", "7"))
QGROUPS = ((0,), (1, 2), (3, 4, 5, 6, 7))


def _pack_rows(x):
    n = x.shape[0] // 16
    x3 = x.reshape(n, 16, x.shape[1])
    w = pltpu.pack_elementwise([x3[:, 0:8, :], x3[:, 8:16, :]], packed_dtype=jnp.bfloat16)
    return w.reshape(n * 8, x.shape[1])


@jax.jit
def pallas_standalone__gqa_block_cached__near_ridge_kernel(x, k_cache, v_cache, wq, wo):
    B, Sq, D = x.shape
    _, Hkv, Sk, Dh = k_cache.shape
    rep = HQ // Hkv
    G = rep * Dh
    M = B * Sq
    R = rep * Sq
    H = Sq // 2
    U = B * Hkv
    scale = (Dh ** -0.5) * math.log2(math.e)
    x2 = x.reshape(M, D)
    k3 = k_cache.reshape(U, Sk, Dh)
    v3 = v_cache.reshape(U, Sk, Dh)
    NT = Sk // 128
    NG = R // RG
    NRND = NT // 4
    NS = (U - 1) // NU
    assert NS * NU == U - 1
    color = [i % 2 for i in range(NU)]
    if NU % 2:
        color[-1] = 2
    color.append(color[0])

    def kernel(x_hbm, k_hbm, v_hbm, wq_hbm, wo_hbm, o_ref,
               x_v, wq_v, wo_v, q_scr, o_scr, s0, s1, p0, p1, p2, kbuf, vbuf, k0buf, vlbuf, sem, ksem, vsem):
        step = pl.program_id(0)
        s_scr = (s0, s1)
        p_scr = (p0, p1, p2)
        z1 = jax.lax.shift_right_logical(step, 10)
        z2 = jax.lax.shift_right_logical(step, 11)
        z3 = jax.lax.shift_right_logical(step, 12)
        never = jnp.broadcast_to(z3, (RG, 128)) > 0

        def kcopy(s, pp):
            return pltpu.make_async_copy(k_hbm.at[pl.ds(NU * s + 1, NU)], kbuf.at[pp], ksem.at[pp])

        def vcopy(s, pp):
            return pltpu.make_async_copy(v_hbm.at[pl.ds(NU * s, NU)], vbuf.at[pp], vsem.at[pp])

        x_copy = pltpu.make_async_copy(x_hbm, x_v, sem.at[0])
        wq_copies = [
            pltpu.make_async_copy(wq_hbm.at[:, grp[0] * G:(grp[-1] + 1) * G],
                                  wq_v.at[:, grp[0] * G:(grp[-1] + 1) * G], sem.at[1 + n])
            for n, grp in enumerate(QGROUPS)]
        nq = len(QGROUPS)
        k0_copy = pltpu.make_async_copy(k_hbm.at[0], k0buf, sem.at[1 + nq])
        vl_copy = pltpu.make_async_copy(v_hbm.at[U - 1], vlbuf, sem.at[2 + nq])
        wo_copy = pltpu.make_async_copy(wo_hbm, wo_v, sem.at[3 + nq])

        def qproj(g):
            q = jnp.dot(x_v[...], wq_v[:, g * G:(g + 1) * G], preferred_element_type=jnp.float32)
            toks = [q[u * RG * 2:u * RG * 2 + RG, r * 128:(r + 1) * 128]
                    for r in range(rep) for u in range(NG)]
            qw = _pack_rows(q * scale)
            for bb in range(B):
                for r in range(rep):
                    q_scr[bb * Hkv + g, r * H:(r + 1) * H, :] = qw[bb * H:(bb + 1) * H, r * Dh:(r + 1) * Dh]
            return toks

        def stage_a(u, k, sr):
            q = pltpu.bitcast(q_scr[u], jnp.bfloat16)
            s = jax.lax.dot_general(
                q, k, (((1,), (1,)), ((), ())), preferred_element_type=jnp.float32)
            sr[z1] = s
            return jnp.broadcast_to(jnp.max(s, axis=-1, keepdims=True), (R, 128))

        def stage_b(sr, pr, m, toks):
            ntok = NG * NSPLIT
            cw = NT // NSPLIT
            for t in range(NG):
                rows = slice(t * RG, (t + 1) * RG)
                l = None
                for h in range(NSPLIT):
                    n = t * NSPLIT + h
                    mt = jnp.where(never, toks[n * PACE // ntok], m[rows])
                    for c in range(h * cw, (h + 1) * cw):
                        p = jnp.exp2(sr[z2, rows, c * 128:(c + 1) * 128] - mt)
                        l = p if l is None else l + p
                        pr[z1, c, t * 8:(t + 1) * 8, :] = _pack_rows(p)
                l = jnp.broadcast_to(jnp.sum(l, axis=-1, keepdims=True), (RG, Dh))
                lu = pltpu.bitcast(l, jnp.uint32)
                half = t // (NG // 2)
                tt = t % (NG // 2)
                pr[z1, NT + half, pl.ds(tt * 16, 8, stride=2), :] = lu[0:8]
                pr[z1, NT + half, pl.ds(tt * 16 + 1, 8, stride=2), :] = lu[8:16]

        def stage_c(u, v_ref, pr):
            o = None
            toks = []
            for rnd in range(NRND):
                p = pltpu.bitcast(
                    jnp.concatenate([pr[z2, c] for c in range(4 * rnd, 4 * rnd + 4)], axis=1), jnp.bfloat16)
                part = jnp.dot(p, v_ref[rnd * 512:(rnd + 1) * 512, :],
                               preferred_element_type=jnp.float32)
                toks += [part[t * RG:(t + 1) * RG, :] for t in range(NG)]
                o = part if o is None else o + part
            l = jnp.concatenate([pr[z2, NT], pr[z2, NT + 1]], axis=0)
            l = pltpu.bitcast(l, jnp.float32)
            r = pl.reciprocal(l, approx=True)
            r = r * (2.0 - l * r)
            o_scr[u] = _pack_rows(o * r)
            return toks

        @pl.when(step == 0)
        def _():
            x_copy.start()
            for c in wq_copies:
                c.start()
            k0_copy.start()
            kcopy(0, 0).start()
            vcopy(0, 0).start()
            x_copy.wait()
            for n, grp in enumerate(QGROUPS):
                wq_copies[n].wait()
                if n == nq - 1:
                    k0_copy.wait()
                    m = stage_a(0, k0buf[...], s0)
                for g in grp:
                    toks = qproj(g)
                    if n == nq - 1 and g == grp[0]:
                        stage_b(s0, p_scr[color[0]], m, toks)

        @pl.when(jnp.logical_and(step >= 1, step <= NS))
        def _():
            s = step - 1
            par = s % 2

            @pl.when(s + 1 < NS)
            def _():
                kcopy(s + 1, 1 - par).start()
                vcopy(s + 1, 1 - par).start()

            @pl.when(s + 1 == NS)
            def _():
                vl_copy.start()
                wo_copy.start()

            kcopy(s, par).wait()
            vcopy(s, par).wait()
            for i in range(NU):
                n = s * NU + i
                m = stage_a(n + 1, kbuf[par, i], s_scr[i % 2])
                toks = stage_c(n, vbuf.at[par, i], p_scr[color[i]])
                stage_b(s_scr[i % 2], p_scr[color[i + 1]], m, toks)

        @pl.when(step == NS + 1)
        def _():
            vl_copy.wait()
            wo_copy.wait()
            stage_c(U - 1, vlbuf, p_scr[color[0]])
            acc = None
            for g in range(Hkv):
                lhs = jnp.concatenate(
                    [jnp.concatenate([o_scr[bb * Hkv + g, r * H:(r + 1) * H, :] for r in range(rep)], axis=1)
                     for bb in range(B)], axis=0)
                part = jnp.dot(pltpu.bitcast(lhs, jnp.bfloat16), wo_v[g * G:(g + 1) * G, :],
                               preferred_element_type=jnp.float32)
                acc = part if acc is None else acc + part
            o_ref[...] = pltpu.bitcast(_pack_rows(acc), jnp.bfloat16)

    pshape = pltpu.VMEM((1, NT + 2, R // 2, 128), jnp.uint32)
    out = pl.pallas_call(
        kernel,
        grid=(NS + 2,),
        in_specs=[pl.BlockSpec(memory_space=pl.ANY)] * 5,
        out_specs=pl.BlockSpec((M, D), lambda s: (0, 0)),
        out_shape=jax.ShapeDtypeStruct((M, D), x.dtype),
        scratch_shapes=[
            pltpu.VMEM((M, D), jnp.bfloat16),
            pltpu.VMEM((D, HQ * Dh), jnp.bfloat16),
            pltpu.VMEM((HQ * Dh, D), jnp.bfloat16),
            pltpu.VMEM((U, R // 2, Dh), jnp.uint32),
            pltpu.VMEM((U, R // 2, Dh), jnp.uint32),
            pltpu.VMEM((1, R, Sk), jnp.float32),
            pltpu.VMEM((1, R, Sk), jnp.float32),
            pshape, pshape, pshape,
            pltpu.VMEM((2, NU, Sk, Dh), jnp.bfloat16),
            pltpu.VMEM((2, NU, Sk, Dh), jnp.bfloat16),
            pltpu.VMEM((Sk, Dh), jnp.bfloat16),
            pltpu.VMEM((Sk, Dh), jnp.bfloat16),
            pltpu.SemaphoreType.DMA((4 + len(QGROUPS),)),
            pltpu.SemaphoreType.DMA((2,)),
            pltpu.SemaphoreType.DMA((2,)),
        ],
        compiler_params=pltpu.CompilerParams(
            dimension_semantics=("arbitrary",),
            vmem_limit_bytes=100 * 1024 * 1024,
        ),
    )(x2, k3, v3, wq, wo)
    return out.reshape(B, Sq, D)
```

```python
import math

import jax
import jax.numpy as jnp
import jax.experimental.pallas as pl
import jax.experimental.pallas.tpu as pltpu

HQ = 32
RG = 8
PACE = 76
NU = 6
NS = 10
QA = 4
QG = (5, 7)
KS = ((0, 128), (128, 256), (256, 512))
NWO = 4
OSPLIT = 2


@jax.jit
def pallas_standalone__gqa_block_cached__near_ridge_kernel(x, k_cache, v_cache, wq, wo):
    B, Sq, D = x.shape
    _, Hkv, Sk, Dh = k_cache.shape
    rep = HQ // Hkv
    G = rep * Dh
    M = B * Sq
    R = rep * Sq
    U = B * Hkv
    scale = (Dh ** -0.5) * math.log2(math.e)
    NT = Sk // 128
    NG = R // RG
    NE = R // 16
    NRND = NT // 4
    NMAIN = NS * NU
    NEK = U - 2 - NMAIN
    NEV = U - NMAIN
    nq, nk = len(QG), len(KS)
    qoff = [QA + sum(QG[:n]) for n in range(nq)]
    WOC = HQ * Dh // NWO
    NON = D // 128
    CA = QA * 256
    MO = M // OSPLIT
    assert NU % 2 == 0 and NEK >= 1 and (QA + sum(QG)) * 256 == HQ * Dh and KS[-1][1] == D
    assert NS >= 2 + NWO and QG[-1] >= 3
    S_K0, S_KE, S_VE, S_WO = 0, 1, 2, 3
    S_X = S_WO + NWO
    S_WA = S_X + nk
    S_WQ = S_WA + nk
    S_K = S_WQ + nq
    S_V = S_K + 1
    S_O = S_V + 1
    NSEM = S_O + NON - 1 + OSPLIT
    tok_ids = [t * PACE // NG for t in range(NG)]

    def kernel(x_hbm, k_hbm, v_hbm, wq_hbm, wo_hbm, o_hbm, *rest):
        x_v = rest[:nk]
        wa_v = rest[nk:2 * nk]
        wq_v = rest[2 * nk:2 * nk + nq]
        (qa_scr, wo_v, q_scr, o_scr, out_v, s0, s1, m0, m1, p0, p1, l0, l1,
         kbuf, vbuf, k0buf, kebuf, vebuf, sem) = rest[2 * nk + nq:]
        s_scr, m_scr, p_scr, l_scr = (s0, s1), (m0, m1), (p0, p1), (l0, l1)
        step = pl.program_id(0)
        z1 = jax.lax.shift_right_logical(step, 10)
        z2 = jax.lax.shift_right_logical(step, 11)
        z3 = jax.lax.shift_right_logical(step, 12)
        never = jnp.broadcast_to(z3, (R, 128)) > 0
        never1 = jnp.broadcast_to(z3, (RG, 128)) > 0

        def kcopy(s, pp):
            return pltpu.make_async_copy(k_hbm.at[pl.ds(NU * s + 2, NU)], kbuf.at[pp], sem.at[S_K])

        def vcopy(s, pp):
            return pltpu.make_async_copy(v_hbm.at[pl.ds(NU * s, NU)], vbuf.at[pp], sem.at[S_V])

        def x_copy(n):
            return pltpu.make_async_copy(x_hbm.at[:, KS[n][0]:KS[n][1]], x_v[n], sem.at[S_X + n])

        def wa_copy(n):
            return pltpu.make_async_copy(wq_hbm.at[KS[n][0]:KS[n][1], 0:CA], wa_v[n], sem.at[S_WA + n])

        def wq_copy(n):
            return pltpu.make_async_copy(
                wq_hbm.at[:, qoff[n] * 256:(qoff[n] + QG[n]) * 256], wq_v[n], sem.at[S_WQ + n])

        def k0_copy():
            return pltpu.make_async_copy(k_hbm.at[0:2], k0buf, sem.at[S_K0])

        def ke_copy():
            return pltpu.make_async_copy(k_hbm.at[U - NEK:U], kebuf, sem.at[S_KE])

        def ve_copy():
            return pltpu.make_async_copy(v_hbm.at[U - NEV:U], vebuf, sem.at[S_VE])

        def wo_copy(c):
            rows = pl.ds(c * WOC, WOC) if isinstance(c, int) else pl.ds(pl.multiple_of(c * WOC, WOC), WOC)
            return pltpu.make_async_copy(wo_hbm.at[rows], wo_v.at[rows], sem.at[S_WO + c])

        def out_copy(nt, h=None):
            cols = slice(nt * 128, (nt + 1) * 128)
            if h is None:
                return pltpu.make_async_copy(out_v.at[nt + z2], o_hbm.at[:, cols], sem.at[S_O + nt])
            rows = slice(h * MO, (h + 1) * MO)
            return pltpu.make_async_copy(out_v.at[nt + z2, rows], o_hbm.at[rows, cols], sem.at[S_O + nt + h])

        def store_q(j, q):
            qb = q.astype(jnp.bfloat16)
            g, hf = j // 2, j % 2
            for bb in range(B):
                q_scr[bb * Hkv + g, :, hf * 256:(hf + 1) * 256] = qb[bb * Sq:(bb + 1) * Sq, :]

        def qproj(j, w):
            xx = jnp.concatenate([xr[...] for xr in x_v], axis=1)
            q = jnp.dot(xx, w, preferred_element_type=jnp.float32)
            store_q(j, q)
            return q

        def stage_a(u, k, cc):
            q = jnp.concatenate([q_scr[u, :, r * Dh:(r + 1) * Dh] for r in range(rep)], axis=0)
            s = jax.lax.dot_general(
                q, k, (((1,), (1,)), ((), ())), preferred_element_type=jnp.float32) * scale
            s_scr[cc][z1] = s
            pm = s[:, 0:128]
            for c in range(1, NT):
                pm = jnp.maximum(pm, s[:, c * 128:(c + 1) * 128])
            m_scr[cc][...] = pm

        def stage_b(cc, tok, last_tok=None):
            m = jnp.broadcast_to(jnp.max(m_scr[cc][...], axis=-1, keepdims=True), (R, 128))
            m = jnp.where(never, tok, m)
            p = jnp.exp2(s_scr[cc][z2] - jnp.concatenate([m] * NT, axis=1))
            l = jnp.broadcast_to(jnp.sum(p, axis=-1, keepdims=True), (R, Dh))
            last = jnp.where(never, l, p[:, Sk - 128:])
            if last_tok is not None:
                last = jnp.concatenate(
                    [last[:R - RG], jnp.where(never1, last_tok, last[R - RG:])], axis=0)
            p_scr[cc][z1] = jnp.concatenate([p[:, :Sk - 128], last], axis=1).astype(jnp.bfloat16)
            l_scr[cc][z1] = l

        def stage_c(u, v_ref, cc):
            parts = [jnp.dot(p_scr[cc][z2, :, rnd * 512:(rnd + 1) * 512],
                             v_ref[rnd * 512:(rnd + 1) * 512, :],
                             preferred_element_type=jnp.float32) for rnd in range(NRND)]
            o = parts[0]
            for part in parts[1:]:
                o = o + part
            l = l_scr[cc][z2]
            r = pl.reciprocal(l, approx=True)
            r = r * (2.0 - l * r)
            o = o * r
            o_scr[u] = jnp.concatenate(
                [o[hh * Sq:(hh + 1) * Sq, :] for hh in range(rep)], axis=1).astype(jnp.bfloat16)
            return jnp.concatenate(
                [parts[e // NE][(e % NE) * 16:(e % NE) * 16 + RG, :] for e in tok_ids], axis=0)

        def prologue():
            for n in range(nk):
                x_copy(n).start()
                wa_copy(n).start()
            for n in range(nq):
                wq_copy(n).start()
            k0_copy().start()
            vcopy(0, 0).start()
            kcopy(0, 0).start()
            for n in range(nk):
                x_copy(n).wait()
                wa_copy(n).wait()
                part = jnp.dot(x_v[n][...], wa_v[n][...], preferred_element_type=jnp.float32)
                if n > 0:
                    part = part + qa_scr[...]
                if n < nk - 1:
                    qa_scr[...] = part
                else:
                    for j in range(QA):
                        store_q(j, part[:, j * 256:(j + 1) * 256])
            for n in range(nq):
                wq_copy(n).wait()
                if n == nq - 1:
                    k0_copy().wait()
                qs = []
                for jj in range(QG[n]):
                    qs.append(qproj(qoff[n] + jj, wq_v[n][:, jj * 256:(jj + 1) * 256]))
                    if n == nq - 1 and jj == 0:
                        stage_a(0, k0buf[0], 0)
                    if n == nq - 1 and jj == 2:
                        tok = jnp.concatenate(
                            [qs[1 + e // (2 * NE)][(e % NE) * 32:(e % NE) * 32 + RG,
                                                   (e // NE % 2) * 128:(e // NE % 2 + 1) * 128]
                             for e in tok_ids], axis=0)
                        stage_b(0, tok)
            stage_a(1, k0buf[1], 1)

        def main(s, carry):
            par = jax.lax.bitwise_and(s, 1)
            kcopy(s, par).wait()
            vcopy(s, par).wait()

            @pl.when(s + 1 < NS)
            def _():
                kcopy(s + 1, 1 - par).start()

            for i in range(NU):
                n = s * NU + i
                tok = stage_c(n, vbuf.at[par, i], i % 2)
                if i == 0:
                    @pl.when(s + 1 < NS)
                    def _():
                        vcopy(s + 1, 1 - par).start()

                    @pl.when(s + 2 == NS)
                    def _():
                        ve_copy().start()
                        ke_copy().start()

                    @pl.when(jnp.logical_and(s >= 2, s < 2 + NWO))
                    def _():
                        wo_copy(s - 2).start()
                stage_b((i + 1) % 2, tok)
                stage_a(n + 2, kbuf[par, i], i % 2)
            return carry

        def epilogue():
            ve_copy().wait()
            ke_copy().wait()
            for c in range(NWO):
                wo_copy(c).wait()

            def oproj(g, nt):
                lhs = jnp.concatenate([o_scr[bb * Hkv + g] for bb in range(B)], axis=0)
                return jnp.dot(lhs, wo_v[g * G:(g + 1) * G, nt * 128:(nt + 1) * 128],
                               preferred_element_type=jnp.float32)

            acc = None
            for i in range(NEV - 1):
                n = NMAIN + i
                tok = stage_c(n, vebuf.at[i], i % 2)
                if i == NEV - 2:
                    acc = oproj(0, 0)
                    stage_b((i + 1) % 2, tok, last_tok=acc[0:RG, :])
                else:
                    stage_b((i + 1) % 2, tok)
                if i < NEK:
                    stage_a(n + 2, kebuf[i], i % 2)
            stage_c(U - 1, vebuf.at[NEV - 1], (NEV - 1) % 2)
            for nt in range(NON):
                for g in range(Hkv):
                    if nt == 0 and g == 0:
                        continue
                    part = oproj(g, nt)
                    acc = part if g == 0 else acc + part
                ob = acc.astype(out_v.dtype)
                if nt < NON - 1:
                    out_v[nt + z1] = ob
                    out_copy(nt).start()
                else:
                    for h in range(OSPLIT):
                        out_v[nt + z1, h * MO:(h + 1) * MO] = ob[h * MO:(h + 1) * MO]
                        out_copy(nt, h).start()
            for nt in range(NON - 1):
                out_copy(nt).wait()
            for h in range(OSPLIT):
                out_copy(NON - 1, h).wait()

        @pl.when(step == 0)
        def _():
            prologue()
            jax.lax.fori_loop(0, NS, main, 0)
            epilogue()

    bf16, f32 = jnp.bfloat16, jnp.float32
    out = pl.pallas_call(
        kernel,
        grid=(2,),
        in_specs=[pl.BlockSpec(memory_space=pl.ANY)] * 5,
        out_specs=pl.BlockSpec(memory_space=pl.ANY),
        out_shape=jax.ShapeDtypeStruct((M, D), x.dtype),
        scratch_shapes=[pltpu.VMEM((M, b - a), bf16) for a, b in KS]
        + [pltpu.VMEM((b - a, CA), bf16) for a, b in KS]
        + [pltpu.VMEM((D, n * 256), bf16) for n in QG]
        + [
            pltpu.VMEM((M, CA), f32),
            pltpu.VMEM((HQ * Dh, D), bf16),
            pltpu.VMEM((U, Sq, G), bf16),
            pltpu.VMEM((U, Sq, G), bf16),
            pltpu.VMEM((NON, M, 128), bf16),
            pltpu.VMEM((1, R, Sk), f32), pltpu.VMEM((1, R, Sk), f32),
            pltpu.VMEM((R, 128), f32), pltpu.VMEM((R, 128), f32),
            pltpu.VMEM((1, R, Sk), bf16), pltpu.VMEM((1, R, Sk), bf16),
            pltpu.VMEM((1, R, Dh), f32), pltpu.VMEM((1, R, Dh), f32),
            pltpu.VMEM((2, NU, Sk, Dh), bf16),
            pltpu.VMEM((2, NU, Sk, Dh), bf16),
            pltpu.VMEM((2, Sk, Dh), bf16),
            pltpu.VMEM((NEK, Sk, Dh), bf16),
            pltpu.VMEM((NEV, Sk, Dh), bf16),
            pltpu.SemaphoreType.DMA((NSEM,)),
        ],
        compiler_params=pltpu.CompilerParams(
            dimension_semantics=("arbitrary",),
            vmem_limit_bytes=100 * 1024 * 1024,
            disable_bounds_checks=True,
            disable_semaphore_checks=True,
        ),
    )(x.reshape(M, D), k_cache.reshape(U, Sk, Dh), v_cache.reshape(U, Sk, Dh), wq, wo)
    return out.reshape(B, Sq, D)
```
